```python
import os as _os
_os.environ.setdefault("JAX_PLATFORMS", "cpu")
import jax
import jax.numpy as jnp

def _softmax(x, axis=-1):
    return jax.nn.softmax(x, axis=axis)
def _gelu(x):
    return jax.nn.gelu(x, approximate=True)
def _silu(x):
    return jax.nn.silu(x)
def _sigmoid(x):
    return jax.nn.sigmoid(x)
def _layernorm(x, axis=-1, eps=1e-5):
    m = jnp.mean(x, axis=axis, keepdims=True)
    v = jnp.var(x, axis=axis, keepdims=True)
    return (x - m) / jnp.sqrt(v + eps)
def _scatter_add(tgt, idx, src, axis=0):
    return tgt.at[idx].add(src)
def _segment_sum(src, seg, n):
    return jax.ops.segment_sum(src, seg, n)
class _Rng:
    def __init__(self, key):
        self._k = key
    def _next(self):
        self._k, sub = jax.random.split(self._k)
        return sub
    def normal(self, shape):
        return jax.random.normal(self._next(), shape, dtype=jnp.bfloat16)
    def randint(self, lo, hi, shape):
        return jax.random.randint(self._next(), shape, lo, hi, dtype=jnp.int32)
    def uniform(self, shape, lo=0.0, hi=1.0):
        return jax.random.uniform(self._next(), shape, jnp.bfloat16, lo, hi)
    def permutation(self, n):
        return jax.random.permutation(self._next(), n)


kernel_name = 'concat_heads__mha_block__linear_attn_block__prompt'

def setup_inputs():
    _rng = _Rng(jax.random.key(int.from_bytes(__import__("os").urandom(4), "little")))
    _w = (lambda a: (lambda t: t.astype(jnp.bfloat16) if jnp.issubdtype(t.dtype, jnp.floating) else t)(jnp.asarray(a)))
    def _A_setup():
        B, S, D, H = 1, 2048, 1024, 32
        return {
            "x": _w((lambda *s: _rng.normal(s) * 0.2)(B, S, D)),
            "wqkv": _w((lambda *s: _rng.normal(s) * 0.2)(D, 3 * D)),
            "wo": _w((lambda *s: _rng.normal(s) * 0.05)(D, D)),
        }
    _A_in = _A_setup()

    def _B_setup():
        B, S, D = 1, 2048, 1024
        return {
            "x": _w((lambda *s: _rng.normal(s) * 0.05)(B, S, D)),
            "wqkv": _w((lambda *s: _rng.normal(s) * 1.6)(D, 3 * D)),
            "wo": _w((lambda *s: _rng.normal(s) * 0.1)(D, D)),
        }
    _B_in = _B_setup()

    return {
        "A_x": _A_in["x"],
        "A_wqkv": _A_in["wqkv"],
        "A_wo": _A_in["wo"],
        "B_x": _B_in["x"],
        "B_wqkv": _B_in["wqkv"],
        "B_wo": _B_in["wo"],
    }

def reference(A_x, A_wqkv, A_wo, B_x, B_wqkv, B_wo):
    def _A_ref(x, wqkv, wo):
        B, S, D = x.shape
        H = 32
        Dh = D // H
        qkv = (lambda x, *d: x.transpose(*d))((x @ wqkv).reshape(B, S, 3, H, Dh), 2, 0, 3, 1, 4)
        q, k, v = qkv[0], qkv[1], qkv[2]
        scores = jnp.einsum("bhqd,bhkd->bhqk", q, k) * (Dh ** -0.5)
        p = _softmax(scores, axis=-1)
        o = jnp.einsum("bhqk,bhkd->bhqd", p, v)
        return (lambda x, *d: x.transpose(*d))(o, 0, 2, 1, 3).reshape(B, S, D) @ wo

    def _B_ref(x, wqkv, wo):
        B, S, D = x.shape
        H = 32; Dh = D // H
        qkv = (lambda x, *d: x.transpose(*d))((x @ wqkv).reshape(B, S, 3, H, Dh), 2, 0, 3, 1, 4)
        q, k, v = qkv[0], qkv[1], qkv[2]
        phi = lambda t: jnp.where(t > 0, t + 1, jnp.exp(t)) + 1e-6
        pq, pk = phi(q), phi(k)
        kv = jnp.einsum("bhsd,bhse->bhde", pk, v)
        z = jnp.einsum("bhsd->bhd", pk)
        num = jnp.einsum("bhqd,bhde->bhqe", pq, kv)
        den = jnp.einsum("bhqd,bhd->bhq", pq, z)[..., None] + 1e-6
        o = num / den
        return (lambda x, *d: x.transpose(*d))(o, 0, 2, 1, 3).reshape(B, S, D) @ wo

    a = _A_ref(A_x, A_wqkv, A_wo)
    b = _B_ref(B_x, B_wqkv, B_wo)
    return jnp.concatenate([a, b], axis=-1)
```

```python
import math

import jax
import jax.numpy as jnp
from jax import lax
import jax.experimental.pallas as pl
import jax.experimental.pallas.tpu as pltpu

S = 2048
D = 1024
H = 32
DH = 32
RB = 512
CK = 128
DELTA = 2
U = 4
D1 = 1
D3 = 3
NT = (((1,), (1,)), ((), ()))
F32 = jnp.float32
BF16 = jnp.bfloat16
QSCALE = (DH ** -0.5) * math.log2(math.e)
NR = S // RB
NC = S // CK
T = NR * H


def _phi(t):
    return jnp.where(t > 0, t + 1.0, jnp.exp(t)) + 1e-6


def _fold(op, x):
    r = x[0:8]
    for i in range(1, x.shape[0] // 8):
        r = op(r, x[8 * i:8 * i + 8])
    return r


def _kernel(ax_hbm, aw_hbm, awo_hbm, bx_hbm, bw_hbm, bwo_hbm, out_hbm,
            ax, aw, awo, bx, bw, bwo, wqt, wvt, wkt, kh, vt, qt, s0, s1, ot,
            kv, zacc, kvz, ostage, flag, sem_in, sem_out):

    def cp_ax(r):
        return pltpu.make_async_copy(ax_hbm.at[pl.ds(r * RB, RB), :], ax.at[pl.ds(r * RB, RB), :], sem_in.at[r])

    def cp_aw(j):
        return pltpu.make_async_copy(aw_hbm.at[:, pl.ds(j * D, D)], aw.at[:, pl.ds(j * D, D)], sem_in.at[NR + j])

    cp_awo = pltpu.make_async_copy(awo_hbm, awo, sem_in.at[NR + 3])
    cp_bx = pltpu.make_async_copy(bx_hbm, bx, sem_in.at[NR + 4])
    cp_bw = pltpu.make_async_copy(bw_hbm, bw, sem_in.at[NR + 5])
    cp_bwo = pltpu.make_async_copy(bwo_hbm, bwo, sem_in.at[NR + 6])

    flag[0] = 0
    cp_ax(0).start()
    cp_aw(1).start()
    cp_aw(0).start()
    cp_aw(2).start()
    cp_aw(1).wait()
    cp_aw(0).wait()
    cp_aw(2).wait()
    for r in range(1, NR):
        cp_ax(r).start()

    def a_k(r, c):
        cp_ax(r).wait()
        r0 = pl.multiple_of(r * RB, RB)
        x = ax[pl.ds(r0, RB), :]
        k = jnp.dot(x, aw[:, D:2 * D], preferred_element_type=F32).astype(BF16)
        for h in range(H):
            kh[h, pl.ds(r0, RB), :] = k[:, h * DH:(h + 1) * DH]
        c0 = pl.multiple_of(r * 256, 256)
        wqt[pl.ds(c0, 256), :] = aw[:, pl.ds(c0, 256)].T
        wvt[pl.ds(c0, 256), :] = aw[:, pl.ds(2 * D + c0, 256)].T
        return c

    lax.fori_loop(0, NR, a_k, 0)

    cp_awo.start()
    cp_bx.start()
    cp_bw.start()
    cp_bwo.start()

    def a_qv(r, c):
        r0 = pl.multiple_of(r * RB, RB)
        x = ax[pl.ds(r0, RB), :]
        v_t = lax.dot_general(wvt[...], x, NT, preferred_element_type=F32)
        vt[:, pl.ds(r0, RB)] = v_t.astype(BF16)
        q_t = lax.dot_general(wqt[...], x, NT, preferred_element_type=F32)
        qt[pl.ds(pl.multiple_of(r * D, D), D), :] = (q_t * QSCALE).astype(BF16)
        return c

    lax.fori_loop(0, NR, a_qv, 0)

    never = jnp.broadcast_to(flag[0], (8, RB)) == 1
    sb = [s0, s1]

    def scores_chunk(t, c, s_ref):
        q_h = qt[pl.ds(pl.multiple_of(t * DH, DH), DH), :]
        k = kh[t % H, pl.ds(c * CK, CK), :]
        s = jnp.dot(k, q_h, preferred_element_type=F32)
        s_ref[pl.ds(c * CK, CK), :] = s
        return _fold(jnp.maximum, s)

    def pv_chunk(t, c, s_ref, mb):
        s = s_ref[pl.ds(c * CK, CK), :]
        p = jnp.exp2(s.reshape(CK // 8, 8, RB) - mb[None]).reshape(CK, RB)
        v = vt[pl.ds(pl.multiple_of((t % H) * DH, DH), DH), pl.ds(c * CK, CK)]
        o = jnp.dot(v, p.astype(BF16), preferred_element_type=F32)
        return _fold(jnp.add, p), o

    def full_max(m):
        return jnp.broadcast_to(jnp.max(m, axis=0, keepdims=True), (8, RB))

    def step(t, par, mb, m, sh, oh):
        s_cur, s_nxt = sb[par], sb[1 - par]
        l = acc = mb_next = None
        for c in range(NC):
            if c < NC - DELTA:
                sm = scores_chunk(jnp.minimum(t + 1, T - 1), c + DELTA, s_nxt)
            else:
                sm = scores_chunk(jnp.minimum(t + 2, T - 1), c - (NC - DELTA), s_cur)
            m = sm if m is None else jnp.maximum(m, sm)
            if c == NC - DELTA - 1:
                mb_next = full_max(m)
                m = None
            mbc = mb
            if len(sh) >= D1:
                mbc = jnp.where(never, sh[-D1], mbc)
            if len(oh) >= D3:
                mbc = jnp.where(never, oh[-D3][0:8], mbc)
            sh.append(sm)
            ls, o = pv_chunk(t, c, s_cur, mbc)
            oh.append(o)
            l = ls if l is None else l + ls
            acc = o if acc is None else acc + o
        lt = jnp.sum(l, axis=0, keepdims=True)
        ot[pl.ds(pl.multiple_of(t * DH, DH), DH), :] = (acc / lt).astype(BF16)
        return mb_next, m

    m = None
    for c in range(NC):
        sm = scores_chunk(0, c, s0)
        m = sm if m is None else jnp.maximum(m, sm)
    mb0 = full_max(m)
    m = None
    for c in range(DELTA):
        sm = scores_chunk(1, c, s1)
        m = sm if m is None else jnp.maximum(m, sm)

    def grp(j, carry):
        mb, m = carry
        sh, oh = [], []
        for u in range(U):
            mb, m = step(U * j + u, u % 2, mb, m, sh, oh)
        return mb, m

    lax.fori_loop(0, T // U, grp, (mb0, m))

    def out_copy(slot, row0, col0):
        return pltpu.make_async_copy(
            ostage.at[slot], out_hbm.at[pl.ds(row0, RB), pl.ds(col0, D)], sem_out.at[slot])

    cp_awo.wait()
    cp_bw.wait()

    def a_out(r, c):
        r0 = pl.multiple_of(r * RB, RB)
        o = ot[pl.ds(pl.multiple_of(r * D, D), D), :].T
        res = jnp.dot(o, awo[...], preferred_element_type=F32)
        c0 = pl.multiple_of(r * 256, 256)
        wkt[pl.ds(c0, 256), :] = bw[:, pl.ds(D + c0, 256)].T
        ostage[r] = res.astype(BF16)
        out_copy(r, r0, 0).start()
        return c

    lax.fori_loop(0, NR, a_out, 0)

    cp_bx.wait()
    cp_bwo.wait()
    kv[...] = jnp.zeros_like(kv)
    zacc[...] = jnp.zeros_like(zacc)

    def b_kv(r, c):
        r0 = pl.multiple_of(r * RB, RB)
        x = bx[pl.ds(r0, RB), :]
        k_t = lax.dot_general(wkt[...], x, NT, preferred_element_type=F32)
        pk_t = _phi(k_t).astype(BF16)
        v = jnp.dot(x, bw[:, 2 * D:3 * D], preferred_element_type=F32).astype(BF16)
        pf = pk_t.astype(F32)
        zs = pf[:, 0:128]
        for t in range(1, RB // 128):
            zs = zs + pf[:, t * 128:(t + 1) * 128]
        zacc[...] += zs
        for g in range(D // 128):
            sl = slice(g * 128, (g + 1) * 128)
            kv[sl, :] += jnp.dot(pk_t[sl, :], v[:, sl], preferred_element_type=F32)
        return c

    lax.fori_loop(0, NR, b_kv, 0)

    row = lax.broadcasted_iota(jnp.int32, (D, 128), 0)
    col = lax.broadcasted_iota(jnp.int32, (D, 128), 1)
    diag = ((row % 128) // DH) == (col // DH)
    z = jnp.sum(zacc[...], axis=1, keepdims=True)
    kvz[:, 0:128] = jnp.where(diag, kv[...], 0.0).astype(BF16)
    kvz[:, 128:256] = jnp.where(diag, z, 0.0).astype(BF16)

    def b_out(r, c):
        r0 = pl.multiple_of(r * RB, RB)
        x = bx[pl.ds(r0, RB), :]
        q = jnp.dot(x, bw[:, 0:D], preferred_element_type=F32)
        pq = _phi(q).astype(BF16)
        outs = []
        for g in range(D // 128):
            sl = slice(g * 128, (g + 1) * 128)
            nd = jnp.dot(pq[:, sl], kvz[sl, :], preferred_element_type=F32)
            outs.append((nd[:, 0:128] / (nd[:, 128:256] + 1e-6)).astype(BF16))
        o = jnp.concatenate(outs, axis=1)
        res = jnp.dot(o, bwo[...], preferred_element_type=F32)
        out_copy(r, r0, 0).wait()
        ostage[r] = res.astype(BF16)
        out_copy(r, r0, D).start()
        return c

    lax.fori_loop(0, NR, b_out, 0)
    for r in range(NR):
        out_copy(r, r * RB, D).wait()


@jax.jit
def pallas_concat_heads__mha_block__linear_attn_block__prompt_kernel(
    A_x: jax.Array,
    A_wqkv: jax.Array,
    A_wo: jax.Array,
    B_x: jax.Array,
    B_wqkv: jax.Array,
    B_wo: jax.Array,
):
    any_spec = pl.BlockSpec(memory_space=pl.ANY)
    out = pl.pallas_call(
        _kernel,
        in_specs=[any_spec] * 6,
        out_specs=any_spec,
        out_shape=jax.ShapeDtypeStruct((S, 2 * D), BF16),
        scratch_shapes=[
            pltpu.VMEM((S, D), BF16),
            pltpu.VMEM((D, 3 * D), BF16),
            pltpu.VMEM((D, D), BF16),
            pltpu.VMEM((S, D), BF16),
            pltpu.VMEM((D, 3 * D), BF16),
            pltpu.VMEM((D, D), BF16),
            pltpu.VMEM((D, D), BF16),
            pltpu.VMEM((D, D), BF16),
            pltpu.VMEM((D, D), BF16),
            pltpu.VMEM((H, S, DH), BF16),
            pltpu.VMEM((D, S), BF16),
            pltpu.VMEM((NR * D, RB), BF16),
            pltpu.VMEM((S, RB), F32),
            pltpu.VMEM((S, RB), F32),
            pltpu.VMEM((NR * D, RB), BF16),
            pltpu.VMEM((D, 128), F32),
            pltpu.VMEM((D, 128), F32),
            pltpu.VMEM((D, 256), BF16),
            pltpu.VMEM((NR, RB, D), BF16),
            pltpu.SMEM((1,), jnp.int32),
            pltpu.SemaphoreType.DMA((NR + 7,)),
            pltpu.SemaphoreType.DMA((NR,)),
        ],
        compiler_params=pltpu.CompilerParams(vmem_limit_bytes=110 * 1024 * 1024),
    )(A_x.reshape(S, D), A_wqkv, A_wo, B_x.reshape(S, D), B_wqkv, B_wo)
    return out.reshape(1, S, 2 * D)
```

```python
import math

import jax
import jax.numpy as jnp
from jax import lax
import jax.experimental.pallas as pl
import jax.experimental.pallas.tpu as pltpu

S = 2048
D = 1024
H = 32
DH = 32
RB = 512
CK = 128
DELTA = 2
U = 8
D1 = 1
D3 = 3
UN_QV = 2
UN_BK = 1
PEEL = 8
NT = (((1,), (1,)), ((), ()))
F32 = jnp.float32
BF16 = jnp.bfloat16
QSCALE = (DH ** -0.5) * math.log2(math.e)
NR = S // RB
NC = S // CK
T = NR * H


def _phi(t):
    return jnp.where(t > 0, t + 1.0, jnp.exp(t)) + 1e-6


def _fold(op, x):
    r = x[0:8]
    for i in range(1, x.shape[0] // 8):
        r = op(r, x[8 * i:8 * i + 8])
    return r


def _aligned(i, n):
    return i if isinstance(i, int) else pl.multiple_of(i, n)


def _loop(n, unroll, body):
    if unroll == n:
        for i in range(n):
            body(i)
        return

    def trip(j, c):
        for u in range(unroll):
            body(j * unroll + u)
        return c

    lax.fori_loop(0, n // unroll, trip, 0)


def _kernel(ax_hbm, aw_hbm, awo_hbm, bx_hbm, bw_hbm, bwo_hbm, out_hbm,
            ax, aw, awo, bx, bw, bwo, wqt, wvt, kh, vt, qt, s0, s1, ot,
            zacc, mm, ostage, flag, sem_x0, sem_x, sem_w, sem_in, sem_oa, sem_ob):

    HB = RB // 2

    def cp_ax(i):
        return pltpu.make_async_copy(ax_hbm.at[pl.ds(i * HB, HB), :], ax.at[pl.ds(i * HB, HB), :], sem_x.at[i])

    def cp_aw(c0, n, i):
        return pltpu.make_async_copy(aw_hbm.at[:, pl.ds(c0, n)], aw.at[:, pl.ds(c0, n)], sem_w.at[i])

    cp_wq = cp_aw(0, D, 4)
    cp_wv = cp_aw(2 * D, D, 5)
    cp_awo = pltpu.make_async_copy(awo_hbm, awo, sem_in.at[0])
    cp_bx = pltpu.make_async_copy(bx_hbm, bx, sem_in.at[1])
    cp_bw = pltpu.make_async_copy(bw_hbm, bw, sem_in.at[2])
    cp_bwo = pltpu.make_async_copy(bwo_hbm, bwo, sem_in.at[3])

    flag[0] = 0

    def k_piece(r0, nr, c0, ncol):
        k = jnp.dot(ax[r0:r0 + nr, :], aw[:, D + c0:D + c0 + ncol], preferred_element_type=F32).astype(BF16)
        for j in range(ncol // DH):
            kh[c0 // DH + j, r0:r0 + nr, :] = k[:, j * DH:(j + 1) * DH]

    def cp_x0(j):
        return pltpu.make_async_copy(ax_hbm.at[pl.ds(0, RB), pl.ds(j * 256, 256)],
                                     ax.at[pl.ds(0, RB), pl.ds(j * 256, 256)], sem_x0.at[j])

    def cp_wk0(j):
        return pltpu.make_async_copy(aw_hbm.at[pl.ds(j * 256, 256), pl.ds(D, D)],
                                     aw.at[pl.ds(j * 256, 256), pl.ds(D, D)], sem_w.at[j])

    cp_x0(0).start()
    cp_wk0(0).start()
    cp_x0(1).start()
    cp_wk0(1).start()
    for j in range(4):
        cp_x0(j).wait()
        cp_wk0(j).wait()
        if j + 2 < 4:
            cp_x0(j + 2).start()
            cp_wk0(j + 2).start()
        else:
            cp_ax(j).start()
        part = jnp.dot(ax[0:RB, j * 256:(j + 1) * 256], aw[j * 256:(j + 1) * 256, D:2 * D],
                       preferred_element_type=F32)
        if j > 0:
            part = part + jnp.concatenate([s0[0:RB, :], s0[RB:2 * RB, :]], axis=1)
        if j < 3:
            s0[0:RB, :] = part[:, 0:RB]
            s0[RB:2 * RB, :] = part[:, RB:2 * RB]
    k = part.astype(BF16)
    for h in range(H):
        kh[h, 0:RB, :] = k[:, h * DH:(h + 1) * DH]
    cp_ax(2).wait()
    cp_ax(3).wait()
    cp_ax(4).start()
    cp_ax(5).start()
    cp_wq.start()
    k_piece(RB, RB, 0, D)
    cp_ax(4).wait()
    cp_ax(5).wait()
    cp_wq.wait()
    cp_ax(6).start()
    cp_ax(7).start()
    cp_wv.start()
    k_piece(2 * RB, RB, 0, D)
    for j in range(4):
        wqt[j * 256:(j + 1) * 256, :] = aw[:, j * 256:(j + 1) * 256].T
    cp_ax(6).wait()
    cp_ax(7).wait()
    cp_wv.wait()
    cp_awo.start()
    cp_bx.start()
    cp_bw.start()
    cp_bwo.start()
    k_piece(3 * RB, RB, 0, D)
    for j in range(4):
        wvt[j * 256:(j + 1) * 256, :] = aw[:, 2 * D + j * 256:2 * D + (j + 1) * 256].T

    def a_qv(r):
        r0 = _aligned(r * RB, RB)
        x = ax[pl.ds(r0, RB), :]
        q_t = lax.dot_general(wqt[...], x, NT, preferred_element_type=F32)
        qt[pl.ds(_aligned(r * D, D), D), :] = (q_t * QSCALE).astype(BF16)
        v_t = lax.dot_general(wvt[...], x, NT, preferred_element_type=F32)
        vt[:, pl.ds(r0, RB)] = v_t.astype(BF16)

    _loop(NR, UN_QV, a_qv)

    never = jnp.broadcast_to(flag[0], (8, RB)) == 1
    sb = [s0, s1]

    def scores_chunk(t, c, s_ref):
        q_h = qt[pl.ds(_aligned(t * DH, DH), DH), :]
        k = kh[t % H, pl.ds(c * CK, CK), :]
        s = jnp.dot(k, q_h, preferred_element_type=F32)
        s_ref[pl.ds(c * CK, CK), :] = s
        return _fold(jnp.maximum, s)

    def pv_chunk(t, c, s_ref, mb):
        s = s_ref[pl.ds(c * CK, CK), :]
        p = jnp.exp2(s.reshape(CK // 8, 8, RB) - mb[None]).reshape(CK, RB)
        v = vt[pl.ds(_aligned((t % H) * DH, DH), DH), pl.ds(c * CK, CK)]
        o = jnp.dot(v, p.astype(BF16), preferred_element_type=F32)
        return _fold(jnp.add, p), o

    def full_max(m):
        return jnp.broadcast_to(jnp.max(m, axis=0, keepdims=True), (8, RB))

    def step(t, par, mb, m, sh, oh, ahead=2):
        s_cur, s_nxt = sb[par], sb[1 - par]
        l = acc = mb_next = None
        for c in range(NC):
            sm = None
            if c < NC - DELTA:
                if ahead >= 1:
                    sm = scores_chunk(t + 1, c + DELTA, s_nxt)
            elif ahead >= 2:
                sm = scores_chunk(t + 2, c - (NC - DELTA), s_cur)
            if sm is not None:
                m = sm if m is None else jnp.maximum(m, sm)
                if c == NC - DELTA - 1:
                    mb_next = full_max(m)
                    m = None
            mbc = mb
            if len(sh) >= D1 and sh[-D1] is not None:
                mbc = jnp.where(never, sh[-D1], mbc)
            if len(oh) >= D3:
                mbc = jnp.where(never, oh[-D3][0:8], mbc)
            elif len(oh) == D3 - 1:
                mbc = jnp.where(never, oh[0][0:8], mbc)
            sh.append(sm)
            ls, o = pv_chunk(t, c, s_cur, mbc)
            oh.append(o)
            l = ls if l is None else l + ls
            acc = o if acc is None else acc + o
        return mb_next, m, l, acc

    def finish(t, l, acc):
        lt = jnp.sum(l, axis=0, keepdims=True)
        ot[pl.ds(_aligned(t * DH, DH), DH), :] = (acc / lt).astype(BF16)

    m = None
    for c in range(NC):
        sm = scores_chunk(0, c, s0)
        m = sm if m is None else jnp.maximum(m, sm)
    mb0 = full_max(m)
    m = None
    for c in range(DELTA):
        sm = scores_chunk(1, c, s1)
        m = sm if m is None else jnp.maximum(m, sm)

    def grp(j, carry):
        mb, m = carry
        sh, oh = [], []
        for u in range(U):
            mb, m, l, acc = step(U * j + u, u % 2, mb, m, sh, oh)
            finish(U * j + u, l, acc)
        return mb, m

    mb, m = lax.fori_loop(0, (T - PEEL) // U, grp, (mb0, m))

    cp_awo.wait()
    cp_bw.wait()

    def out_a(r):
        return pltpu.make_async_copy(ostage.at[r], out_hbm.at[pl.ds(r * RB, RB), pl.ds(0, D)], sem_oa.at[r])

    def out_b(r0, n, i):
        return pltpu.make_async_copy(ax.at[pl.ds(r0, n), :], out_hbm.at[pl.ds(r0, n), pl.ds(D, D)], sem_ob.at[i])

    def a_out(r):
        o = ot[r * D:(r + 1) * D, :].T
        res = jnp.dot(o, awo[...], preferred_element_type=F32)
        c0 = r * 256
        wqt[c0:c0 + 256, :] = bw[:, c0:c0 + 256].T
        wvt[c0:c0 + 256, :] = bw[:, D + c0:D + c0 + 256].T
        ostage[r] = res.astype(BF16)

    sh, oh = [], []
    for t in range(T - PEEL, T):
        if t == T - 1:
            a_out(0)
        mb, m, l, acc = step(t, t % 2, mb, m, sh, oh, ahead=T - 1 - t)
        finish(t, l, acc)
    out_a(0).start()
    for r in range(1, NR):
        a_out(r)
        out_a(r).start()

    cp_bx.wait()
    cp_bwo.wait()
    zacc[...] = jnp.zeros_like(zacc)
    pkt = vt
    bv = ax

    def b_k(r):
        r0 = _aligned(r * RB, RB)
        x = bx[pl.ds(r0, RB), :]
        k_t = lax.dot_general(wvt[...], x, NT, preferred_element_type=F32)
        pf = _phi(k_t)
        pkt[:, pl.ds(r0, RB)] = pf.astype(BF16)
        zs = pf[:, 0:128]
        for t in range(1, RB // 128):
            zs = zs + pf[:, t * 128:(t + 1) * 128]
        zacc[...] += zs
        bv[pl.ds(r0, RB), :] = jnp.dot(x, bw[:, 2 * D:3 * D], preferred_element_type=F32).astype(BF16)

    _loop(NR, UN_BK, b_k)

    row = lax.broadcasted_iota(jnp.int32, (128, 128), 0)
    col = lax.broadcasted_iota(jnp.int32, (128, 128), 1)
    diag = (row // DH) == (col // DH)

    zacc[...] = jnp.broadcast_to(jnp.sum(zacc[...], axis=1, keepdims=True), (D, 128))
    for g in range(D // 128):
        sl = slice(g * 128, (g + 1) * 128)
        kv_g = jnp.dot(pkt[sl, :], bv[:, sl], preferred_element_type=F32)
        kv_g = jnp.where(diag, kv_g, 0.0).astype(BF16)
        mm[sl, :] = jnp.dot(kv_g, bwo[sl, :], preferred_element_type=F32).astype(BF16)

    def b_out(r, split):
        r0 = _aligned(r * RB, RB)
        x = bx[pl.ds(r0, RB), :]
        q_t = lax.dot_general(wqt[...], x, NT, preferred_element_type=F32)
        pq = _phi(q_t)
        zb = zacc[...]
        w = pq * jnp.concatenate([zb] * (RB // 128), axis=1)
        den = jnp.sum(w.reshape(H, DH, RB), axis=1, keepdims=True) + 1e-6
        o_t = (pq.reshape(H, DH, RB) * (1.0 / den)).reshape(D, RB).astype(BF16)
        o = o_t.T
        if split:
            for i in range(2):
                res = jnp.dot(o[i * HB:(i + 1) * HB], mm[...], preferred_element_type=F32)
                r1 = _aligned(r0 + i * HB, HB)
                ax[pl.ds(r1, HB), :] = res.astype(BF16)
                out_b(r1, HB, 2 * r + i).start()
        else:
            res = jnp.dot(o, mm[...], preferred_element_type=F32)
            ax[pl.ds(r0, RB), :] = res.astype(BF16)
            out_b(r0, RB, 2 * r).start()

    def b_pair(j):
        b_out(2 * j, False)
        b_out(2 * j + 1, True)

    _loop(NR // 2, 1, b_pair)
    for r in range(NR):
        out_a(r).wait()
        if r % 2 == 0:
            out_b(r * RB, RB, 2 * r).wait()
        else:
            out_b(r * RB, HB, 2 * r).wait()
            out_b(r * RB + HB, HB, 2 * r + 1).wait()


@jax.jit
def pallas_concat_heads__mha_block__linear_attn_block__prompt_kernel(
    A_x: jax.Array,
    A_wqkv: jax.Array,
    A_wo: jax.Array,
    B_x: jax.Array,
    B_wqkv: jax.Array,
    B_wo: jax.Array,
):
    any_spec = pl.BlockSpec(memory_space=pl.ANY)
    out = pl.pallas_call(
        _kernel,
        in_specs=[any_spec] * 6,
        out_specs=any_spec,
        out_shape=jax.ShapeDtypeStruct((S, 2 * D), BF16),
        scratch_shapes=[
            pltpu.VMEM((S, D), BF16),
            pltpu.VMEM((D, 3 * D), BF16),
            pltpu.VMEM((D, D), BF16),
            pltpu.VMEM((S, D), BF16),
            pltpu.VMEM((D, 3 * D), BF16),
            pltpu.VMEM((D, D), BF16),
            pltpu.VMEM((D, D), BF16),
            pltpu.VMEM((D, D), BF16),
            pltpu.VMEM((H, S, DH), BF16),
            pltpu.VMEM((D, S), BF16),
            pltpu.VMEM((NR * D, RB), BF16),
            pltpu.VMEM((S, RB), F32),
            pltpu.VMEM((S, RB), F32),
            pltpu.VMEM((NR * D, RB), BF16),
            pltpu.VMEM((D, 128), F32),
            pltpu.VMEM((D, D), BF16),
            pltpu.VMEM((NR, RB, D), BF16),
            pltpu.SMEM((1,), jnp.int32),
            pltpu.SemaphoreType.DMA((4,)),
            pltpu.SemaphoreType.DMA((2 * NR,)),
            pltpu.SemaphoreType.DMA((6,)),
            pltpu.SemaphoreType.DMA((4,)),
            pltpu.SemaphoreType.DMA((NR,)),
            pltpu.SemaphoreType.DMA((2 * NR,)),
        ],
        compiler_params=pltpu.CompilerParams(vmem_limit_bytes=110 * 1024 * 1024),
    )(A_x.reshape(S, D), A_wqkv, A_wo, B_x.reshape(S, D), B_wqkv, B_wo)
    return out.reshape(1, S, 2 * D)
```
